```python
import os as _os
_os.environ.setdefault('JAX_PLATFORMS', 'cpu')
import jax
import jax.numpy as jnp

def _softmax(x, axis=-1):
    return jax.nn.softmax(x, axis=axis)

def _gelu(x):
    return jax.nn.gelu(x, approximate=True)

def _silu(x):
    return jax.nn.silu(x)

def _sigmoid(x):
    return jax.nn.sigmoid(x)

def _layernorm(x, axis=-1, eps=1e-05):
    m = jnp.mean(x, axis=axis, keepdims=True)
    v = jnp.var(x, axis=axis, keepdims=True)
    return (x - m) / jnp.sqrt(v + eps)

def _scatter_add(tgt, idx, src, axis=0):
    return tgt.at[idx].add(src)

def _segment_sum(src, seg, n):
    return jax.ops.segment_sum(src, seg, n)

class _Rng:

    def __init__(self, key):
        self._k = key

    def _next(self):
        self._k, sub = jax.random.split(self._k)
        return sub

    def normal(self, shape):
        return jax.random.normal(self._next(), shape, dtype=jnp.bfloat16)

    def randint(self, lo, hi, shape):
        return jax.random.randint(self._next(), shape, lo, hi, dtype=jnp.int32)

    def uniform(self, shape, lo=0.0, hi=1.0):
        return jax.random.uniform(self._next(), shape, jnp.bfloat16, lo, hi)

    def permutation(self, n):
        return jax.random.permutation(self._next(), n)
kernel_name = 'concat_heads__linear_kernel_hedgehog__memory_aug_recurrent_mem_tr__prompt'

def setup_inputs():
    _rng = _Rng(jax.random.key(int.from_bytes(__import__("os").urandom(4), "little")))
    _w = lambda a: (lambda t: t.astype(jnp.bfloat16) if jnp.issubdtype(t.dtype, jnp.floating) else t)(jnp.asarray(a))

    def _A_setup():
        B, S, D, H = (1, 2048, 576, 32)
        Dh = D // H
        return {'x': _w((lambda *s: _rng.normal(s) * 0.4)(B, S, D)), 'wqkv': _w((lambda *s: _rng.normal(s) * 0.4)(D, 3 * D)), 'w_phi': _w((lambda *s: _rng.normal(s) * 0.4)(H, Dh, Dh) * Dh ** (-0.5)), 'wo': _w((lambda *s: _rng.normal(s) * 0.05)(D, D))}
    _A_in = _A_setup()

    def _B_setup():
        B, S, Dm = (1, 2048, 576)
        H, Dh = (32, 128)
        M, seg = (8, 32)
        seg = min(seg, S)
        S = S // seg * seg
        return {'x': _w((lambda *s: _rng.normal(s) * 0.05)(B, S, Dm)), 'mem0': _w((lambda *s: _rng.normal(s) * 0.8)(B, M, Dm)), 'Wq': _w((lambda *s: _rng.normal(s) * 3.2)(Dm, H, Dh) * Dm ** (-0.5)), 'Wk': _w((lambda *s: _rng.normal(s) * 3.2)(Dm, H, Dh) * Dm ** (-0.5)), 'Wv': _w((lambda *s: _rng.normal(s) * 0.8)(Dm, H, Dh) * Dm ** (-0.5)), 'Wo': _w((lambda *s: _rng.normal(s) * 0.8)(H, Dh, Dm) * (H * Dh) ** (-0.5)), 'seg_len': seg}
    _B_in = _B_setup()
    return {'A_x': _A_in['x'], 'A_wqkv': _A_in['wqkv'], 'A_w_phi': _A_in['w_phi'], 'A_wo': _A_in['wo'], 'B_x': _B_in['x'], 'B_mem0': _B_in['mem0'], 'B_Wq': _B_in['Wq'], 'B_Wk': _B_in['Wk'], 'B_Wv': _B_in['Wv'], 'B_Wo': _B_in['Wo'], 'B_seg_len': _B_in['seg_len']}

def reference(A_x, A_wqkv, A_w_phi, A_wo, B_x, B_mem0, B_Wq, B_Wk, B_Wv, B_Wo, B_seg_len):

    def _A_ref(x, wqkv, w_phi, wo):
        B, S, D = x.shape
        H = 32
        Dh = D // H
        qkv = (lambda x, *d: x.transpose(*d))((x @ wqkv).reshape(B, S, 3, H, Dh), 2, 0, 3, 1, 4)
        q, k, v = (qkv[0], qkv[1], qkv[2])
        pq = jnp.einsum('bhsd,hdf->bhsf', q, w_phi)
        pk = jnp.einsum('bhsd,hdf->bhsf', k, w_phi)
        phi_q = jnp.concatenate([_softmax(pq, axis=-1), _softmax(-pq, axis=-1)], axis=-1)
        phi_k = jnp.concatenate([_softmax(pk, axis=-1), _softmax(-pk, axis=-1)], axis=-1)
        kv = jnp.einsum('bhsf,bhsd->bhfd', phi_k, v)
        z = jnp.einsum('bhsf->bhf', phi_k)
        num = jnp.einsum('bhqf,bhfd->bhqd', phi_q, kv)
        den = jnp.einsum('bhqf,bhf->bhq', phi_q, z)[..., None] + 1e-06
        o = num / den
        return (lambda x, *d: x.transpose(*d))(o, 0, 2, 1, 3).reshape(B, S, D) @ wo

    def _B_ref(x, mem0, Wq, Wk, Wv, Wo, seg_len):
        B, S, Dm = x.shape
        H, Dh = (Wq.shape[1], Wq.shape[2])
        M = mem0.shape[1]
        scale = Dh ** (-0.5)
        n_seg = S // seg_len
        L = M + seg_len
        idx = jnp.arange(L)
        mask = (idx[:, None] < M) | (idx[:, None] >= idx[None, :])
        mem = mem0
        outs = []
        for s in range(n_seg):
            xs = x[:, s * seg_len:(s + 1) * seg_len, :].copy()
            h = jnp.concatenate([mem, xs], axis=1)
            q = jnp.einsum('btd,dhe->bhte', h, Wq)
            k = jnp.einsum('btd,dhe->bhte', h, Wk)
            v = jnp.einsum('btd,dhe->bhte', h, Wv)
            scores = jnp.einsum('bhqe,bhke->bhqk', q, k) * scale
            scores = jnp.where(mask[None, None], scores, -1000000000.0)
            p = _softmax(scores, axis=-1)
            o = jnp.einsum('bhqk,bhke->bhqe', p, v)
            o = jnp.einsum('bhte,hed->btd', o, Wo)
            mem = o[:, :M, :].copy()
            outs.append(o[:, M:, :])
        return jnp.concatenate(outs, axis=1)
    a = _A_ref(A_x, A_wqkv, A_w_phi, A_wo)
    b = _B_ref(B_x, B_mem0, B_Wq, B_Wk, B_Wv, B_Wo, B_seg_len)
    return jnp.concatenate([a, b], axis=-1)
```

```python
import functools
import math

import jax
import jax.numpy as jnp
from jax import lax
import jax.experimental.pallas as pl
import jax.experimental.pallas.tpu as pltpu

F32 = jnp.float32
BF16 = jnp.bfloat16

S = 2048
D = 576
H = 32
DA = 18
DB = 128
MEM = 8
SEG = 32
NG = 4
GR = 8 * DA
T1 = 256
T2 = 128

_NT = (((1,), (1,)), ((), ()))


def _dot(a, b):
    return jnp.dot(a, b, preferred_element_type=F32)


def _dot_nt(a, b):
    return lax.dot_general(a, b, _NT, preferred_element_type=F32)


def _iota(shape, dim):
    return lax.broadcasted_iota(jnp.int32, shape, dim)


def _ktiles(ref, rows):
    parts = [ref[t, rows, :] for t in range(4)] + [ref[4, rows, 0:64]]
    return jnp.concatenate(parts, axis=1)


def _store_ktiles(ref, rows, val):
    for t in range(4):
        ref[t, rows, :] = val[:, 128 * t:128 * (t + 1)]
    ref[4, rows, 0:64] = val[:, 512:576]


def _hedgehog_exp(p):
    sl = [p[8 * f:8 * f + 8, :] for f in range(DA)]
    mx = functools.reduce(jnp.maximum, sl)
    mn = functools.reduce(jnp.minimum, sl)
    ep = [jnp.exp(s - mx) for s in sl]
    en = [jnp.exp(mn - s) for s in sl]
    sp = functools.reduce(jnp.add, ep)
    sn = functools.reduce(jnp.add, en)
    return ep, en, sp, sn


def _kernel(axT_h, awqkv_h, wphi_h, awo_h, bxT_h, mem0_h, wq_h, wk_h, wv_h, woT_h,
            out_h,
            axT, awqkv, wphi, awo, bxT, mem0, wstage, woT_st,
            w2d, wT, kvacc, zacc, kvwoT, bx, wqkv_s, wo_s, fmask, outv,
            st_qkv, st_o, phiq,
            sem_in, sem_out):
    srcs = [wphi_h, awqkv_h, axT_h, awo_h, mem0_h, bxT_h, woT_h, wq_h, wk_h, wv_h]
    dsts = [wphi, awqkv, axT, awo, mem0, bxT, woT_st,
            wstage.at[0], wstage.at[1], wstage.at[2]]
    cps = [pltpu.make_async_copy(s, d, sem_in.at[i])
           for i, (s, d) in enumerate(zip(srcs, dsts))]
    (c_wphi, c_awqkv, c_axT, c_awo, c_mem0, c_bxT, c_woT, c_wq, c_wk, c_wv) = cps
    for c in cps:
        c.start()

    ri = _iota((80, 80), 0)
    ci = _iota((80, 80), 1)
    head_r = ((ri >= 32) & (ri < 64)) | (ri >= 72)
    head_c = ((ci >= 32) & (ci < 64)) | (ci >= 72)
    same = head_r == head_c
    vis = (ri >= 64) | (ci >= 64) | ((ci & 31) <= (ri & 31))
    scale = DB ** -0.5
    fmask[...] = jnp.where(same, jnp.where(vis, 0.0, -1e9 / scale), -jnp.inf).astype(F32)

    w2d[...] = jnp.zeros(w2d.shape, F32)
    kvacc[...] = jnp.zeros(kvacc.shape, F32)
    zacc[...] = jnp.zeros(zacc.shape, F32)
    c_wphi.wait()
    eye32 = (_iota((H, H), 0) == _iota((H, H), 1)).astype(BF16)
    for d in range(DA):
        w2d[pl.ds(64 + d, H, stride=DA), 0:DA] = _dot_nt(eye32, wphi[d])
    w2b = w2d[...].astype(BF16)
    e2 = ((_iota((GR, 128), 0) >> 3) == _iota((GR, 128), 1)).astype(BF16)
    rj = _iota((GR, 256), 0) & 7
    cc = _iota((GR, 256), 1)
    c_awqkv.wait()
    for g in range(NG):
        lo = (8 * g + rj) * DA
        for base, woff, coff in ((0, 64, 0), (2 * D, 0, 512)):
            hd = cc + (128 * g + woff - 64)
            bdt = _dot_nt(e2, w2b[128 * g + woff:128 * g + woff + 256, :])
            bdt = jnp.where((hd >= lo) & (hd < lo + DA), bdt, 0.0).astype(BF16)
            wfold = _dot_nt(bdt, awqkv[:, coff + 128 * g:coff + 128 * g + 256])
            _store_ktiles(wT, slice(base + GR * g, base + GR * (g + 1)), wfold.astype(BF16))
    eye128 = (_iota((128, 128), 0) == _iota((128, 128), 1)).astype(BF16)
    for t in range(5):
        n = 128 if t < 4 else 64
        vt = _dot_nt(eye128[0:n, 0:n], awqkv[:, 2 * D + 128 * t:2 * D + 128 * t + n])
        _store_ktiles(wT, slice(D + 128 * t, D + 128 * t + n), vt.astype(BF16))

    c_axT.wait()

    def phase1(i, carry):
        xw = axT[:, pl.ds(pl.multiple_of(i * T1, T1), T1)]
        vT = _dot(_ktiles(wT, slice(D, 2 * D)), xw).astype(BF16)
        for g in range(NG):
            pk = _dot(_ktiles(wT, slice(2 * D + GR * g, 2 * D + GR * (g + 1))), xw)
            ep, en, sp, sn = _hedgehog_exp(pk)
            rp = 1.0 / sp
            rn = 1.0 / sn
            phi = jnp.concatenate([e * rp for e in ep] + [e * rn for e in en], axis=0)
            n = 256 if g < 3 else 192
            kvacc[g, :, 0:n] += _dot_nt(phi.astype(BF16), vT[128 * g:128 * g + n, :])
            zacc[288 * g:288 * (g + 1), :] += phi[:, 0:128] + phi[:, 128:256]
        return carry

    lax.fori_loop(0, S // T1, phase1, 0)

    c_awo.wait()
    rj2 = _iota((288, 256), 0) & 7
    cc2 = _iota((288, 256), 1)
    kws = []
    for g in range(NG):
        n = 256 if g < 3 else 192
        lo = (8 * g + rj2) * DA - 128 * g
        kvm = jnp.where((cc2 >= lo) & (cc2 < lo + DA), kvacc[g], 0.0).astype(BF16)
        kws.append(_dot(kvm[:, 0:n], awo[128 * g:128 * g + n, :]))
    kw = jnp.concatenate(kws, axis=0)
    kw = jnp.concatenate([kw, kw[:, 512:576]], axis=1)
    for t in range(9):
        kvwoT[t] = kw[128 * t:128 * (t + 1), :].T[0:D, :].astype(BF16)
    zacc[...] = jnp.broadcast_to(jnp.sum(zacc[...], axis=1, keepdims=True), zacc.shape)

    c_bxT.wait()

    def xpose_x(i, carry):
        r0 = pl.multiple_of(i * 128, 128)
        blk = bxT[:, pl.ds(r0, 128)]
        for t in range(4):
            bx[t, pl.ds(r0, 128), :] = blk[128 * t:128 * (t + 1), :].T
        bx[4, pl.ds(r0, 128), :] = jnp.concatenate([blk[512:576, :], blk[512:576, :]], axis=0).T
        return carry

    lax.fori_loop(0, S // 128, xpose_x, 0)

    c_woT.wait()

    def xpose_wo(h, carry):
        r0 = pl.multiple_of(h * 128, 128)
        blk = woT_st[h]
        for t in range(4):
            wo_s[t, pl.ds(r0, 128), :] = blk[128 * t:128 * (t + 1), :].T
        wo_s[4, pl.ds(r0, 128), :] = jnp.concatenate([blk[512:576, :], blk[512:576, :]], axis=0).T
        return carry

    lax.fori_loop(0, H, xpose_wo, 0)

    s32 = wstage.bitcast(jnp.uint32)
    for w, cp in enumerate((c_wq, c_wk, c_wv)):
        cp.wait()

        def relayout(c, carry, w=w):
            sub = s32.at[w, pl.ds(pl.multiple_of(c * 1024, 1024), 1024)]
            r0 = pl.multiple_of(c * 64, 64)
            for i in range(16):
                u = sub[pl.ds(i, 64, stride=16), :]
                lo = pltpu.bitcast(u << 16, F32).astype(BF16)
                hi = pltpu.bitcast(u & jnp.uint32(0xFFFF0000), F32).astype(BF16)
                wqkv_s[6 * i + 2 * w, pl.ds(r0, 64), :] = lo
                wqkv_s[6 * i + 2 * w + 1, pl.ds(r0, 64), :] = hi
            return carry

        lax.fori_loop(0, 9, relayout, 0)

    c_mem0.wait()

    cexp = scale * math.log2(math.e)

    def stack(a, b):
        return jnp.concatenate([a[0], b[0], a[1], b[1]], axis=0).astype(BF16)

    def scores(q2, k2):
        s = _dot_nt(q2, k2)
        fm = fmask[...]
        s = jnp.where(fm == 0.0, s, fm)
        m = jnp.max(s, axis=1, keepdims=True)
        p = jnp.exp2((s - m) * cexp)
        l = jnp.sum(p, axis=1, keepdims=True)
        return p.astype(BF16), 1.0 / l

    def out_proj(lhs, hp):
        rows = slice(256 * hp, 256 * (hp + 1))
        parts = [_dot(lhs, wo_s[t, rows, :]) for t in range(4)]
        parts.append(_dot(lhs, wo_s[4, rows, 0:64]))
        return jnp.concatenate(parts, axis=1)

    def b_step(lhs, first, fillers):
        qk, vv, pp, oo = {}, {}, {}, {}
        acc = [None]

        def proj(hp, t):
            a = _dot(lhs, wqkv_s[6 * hp + t])
            if first:
                st_qkv[6 * hp + t] = a[32:40]
                return a[0:32], a[40:48]
            return jnp.concatenate([st_qkv[6 * hp + t], a[8:32]], axis=0), a[0:8]

        def st_s(hp):
            if 0 <= hp < 16:
                pp[hp] = scores(*qk.pop(hp))

        def st_pv(hp):
            if 0 <= hp < 16:
                p, rl = pp.pop(hp)
                o = _dot(p, vv.pop(hp)) * rl
                halves = []
                for j, (ox, om) in enumerate(((o[0:32], o[64:72]), (o[32:64], o[72:80]))):
                    if first:
                        st_o[2 * hp + j] = ox[24:32]
                        halves.append(jnp.concatenate([ox[0:24], om], axis=0))
                    else:
                        halves.append(jnp.concatenate([st_o[2 * hp + j], ox, om], axis=0))
                oo[hp] = jnp.concatenate(halves, axis=1).astype(BF16)

        def st_o_(hp):
            if 0 <= hp < 16:
                c = out_proj(oo.pop(hp), hp)
                acc[0] = c if acc[0] is None else acc[0] + c

        fillers = list(fillers)
        for t in range(16):
            q = stack(proj(t, 0), proj(t, 1))
            st_s(t - 1)
            k = stack(proj(t, 2), proj(t, 3))
            qk[t] = (q, k)
            st_pv(t - 2)
            vv[t] = stack(proj(t, 4), proj(t, 5))
            st_o_(t - 3)

        def fill():
            if fillers:
                fillers.pop(0)()

        st_pv(14)
        st_o_(13)
        st_s(15)
        st_o_(14)
        fill()
        st_pv(15)
        fill()
        st_o_(15)
        while fillers:
            fill()
        return acc[0]

    def b_pair(r0, mem, fill1, fill2):
        x48 = _ktiles(bx, pl.ds(r0, 48)).astype(F32)
        x16 = _ktiles(bx, pl.ds(r0 + 48, 16)).astype(F32)
        lhs = jnp.concatenate([x48[0:40], mem], axis=0).astype(BF16)
        acc = b_step(lhs, True, fill1)
        b1 = acc[0:24]
        mem = acc[24:32].astype(BF16).astype(F32)
        lhs = jnp.concatenate([mem, x48[40:48], x16], axis=0).astype(BF16)
        acc = b_step(lhs, False, fill2)
        b = jnp.concatenate([b1, acc[0:40]], axis=0)
        return b, acc[40:48].astype(BF16).astype(F32)

    def a_phi(r0, g):
        xw = axT[:, pl.ds(r0, T2)]
        pq = _dot(_ktiles(wT, slice(GR * g, GR * (g + 1))), xw)
        ep, en, sp, sn = _hedgehog_exp(pq)
        z = zacc[288 * g:288 * (g + 1), :]
        dp = functools.reduce(jnp.add, [e * z[8 * f:8 * f + 8] for f, e in enumerate(ep)])
        dn = functools.reduce(jnp.add, [e * z[GR + 8 * f:GR + 8 * f + 8] for f, e in enumerate(en)])
        rp = 1.0 / sp
        rn = 1.0 / sn
        rden = 1.0 / (dp * rp + dn * rn + 1e-06)
        cp_ = rp * rden
        cn_ = rn * rden
        phiq[288 * g:288 * (g + 1), :] = jnp.concatenate(
            [e * cp_ for e in ep] + [e * cn_ for e in en], axis=0).astype(BF16)

    def a_out(r0, c):
        n = 128 if c < 4 else 64
        lhs = jnp.concatenate([kvwoT[t, 128 * c:128 * c + n, :] for t in range(9)], axis=1)
        oT = _dot(lhs, phiq[...])
        if n == 64:
            oT = jnp.concatenate([oT, oT], axis=0)
        outv[pl.ds(r0, T2), 128 * c:128 * c + n] = oT.T[:, 0:n].astype(BF16)

    def out_copy(i):
        rows = pl.ds(pl.multiple_of(i * T2, T2), T2)
        return pltpu.make_async_copy(outv.at[rows], out_h.at[rows], sem_out.at[i])

    for g in range(NG):
        a_phi(0, g)

    def main(i, mem):
        r0 = pl.multiple_of(i * T2, T2)
        rn = pl.multiple_of(jnp.minimum(i + 1, S // T2 - 1) * T2, T2)
        P = functools.partial
        b1, mem = b_pair(r0, mem, [P(a_out, r0, 0), P(a_out, r0, 4)],
                         [P(a_out, r0, 1), P(a_out, r0, 2)])
        outv[pl.ds(r0, 64), D:2 * D] = b1.astype(BF16)
        b2, mem = b_pair(r0 + 64, mem, [P(a_out, r0, 3), P(a_phi, rn, 0)],
                         [P(a_phi, rn, 1), P(a_phi, rn, 2), P(a_phi, rn, 3)])
        outv[pl.ds(r0 + 64, 64), D:2 * D] = b2.astype(BF16)
        out_copy(i).start()
        return mem

    lax.fori_loop(0, S // T2, main, mem0[...].astype(F32))
    for i in range(S // T2):
        out_copy(i).wait()


@functools.partial(jax.jit, static_argnames=("B_seg_len",))
def pallas_concat_heads__linear_kernel_hedgehog__memory_aug_recurrent_mem_tr__prompt_kernel(
    A_x: jax.Array,
    A_wqkv: jax.Array,
    A_w_phi: jax.Array,
    A_wo: jax.Array,
    B_x: jax.Array,
    B_mem0: jax.Array,
    B_Wq: jax.Array,
    B_Wk: jax.Array,
    B_Wv: jax.Array,
    B_Wo: jax.Array,
    B_seg_len: int,
):
    assert int(B_seg_len) == SEG
    assert A_x.shape == (1, S, D) and B_x.shape == (1, S, D)
    args = (
        A_x[0].T,
        A_wqkv,
        jnp.transpose(A_w_phi, (1, 2, 0)),
        A_wo,
        B_x[0].T,
        B_mem0[0],
        B_Wq.reshape(D * H, DB),
        B_Wk.reshape(D * H, DB),
        B_Wv.reshape(D * H, DB),
        jnp.transpose(B_Wo, (0, 2, 1)),
    )
    hbm = pl.BlockSpec(memory_space=pltpu.HBM)
    out = pl.pallas_call(
        _kernel,
        out_shape=jax.ShapeDtypeStruct((S, 2 * D), BF16),
        in_specs=[hbm] * len(args),
        out_specs=hbm,
        scratch_shapes=[
            pltpu.VMEM((D, S), BF16),
            pltpu.VMEM((D, 3 * D), BF16),
            pltpu.VMEM((DA, DA, H), BF16),
            pltpu.VMEM((D, D), BF16),
            pltpu.VMEM((D, S), BF16),
            pltpu.VMEM((MEM, D), BF16),
            pltpu.VMEM((3, D * H, DB), BF16),
            pltpu.VMEM((H, D, DB), BF16),
            pltpu.VMEM((704, 128), F32),
            pltpu.VMEM((5, 3 * D, 128), BF16),
            pltpu.VMEM((NG, 288, 256), F32),
            pltpu.VMEM((2 * D, 128), F32),
            pltpu.VMEM((9, D, 128), BF16),
            pltpu.VMEM((5, S, 128), BF16),
            pltpu.VMEM((96, D, DB), BF16),
            pltpu.VMEM((5, H * DB, 128), BF16),
            pltpu.VMEM((80, 80), F32),
            pltpu.VMEM((S, 2 * D), BF16),
            pltpu.VMEM((96, 8, 128), F32),
            pltpu.VMEM((32, 8, 128), F32),
            pltpu.VMEM((2 * D, T2), BF16),
            pltpu.SemaphoreType.DMA((10,)),
            pltpu.SemaphoreType.DMA((S // T2,)),
        ],
        compiler_params=pltpu.CompilerParams(vmem_limit_bytes=100 * 1024 * 1024),
    )(*args)
    return out.reshape(1, S, 2 * D)
```

```python
import functools
import math

import jax
import jax.numpy as jnp
from jax import lax
import jax.experimental.pallas as pl
import jax.experimental.pallas.tpu as pltpu

F32 = jnp.float32
BF16 = jnp.bfloat16
U32 = jnp.uint32

S = 2048
D = 576
H = 32
DA = 18
DB = 128
MEM = 8
SEG = 32
NG = 4
GR = 8 * DA
T1 = 256
N1 = S // T1
T2 = 128
N2 = S // T2
WCH = 192
PQA = 1

_EVEN = (1, 3, 0, 10, 0, 'S15 O6 P13 O7 P14 O8 O9 O10 P15 M O11 O12 O13 O14 O15')
_ODD = (2, 6, 1, 7, 0, 'S14 V15 P10 S15 P11 O9 P12 P13 O10 P14 O11 P15 M O12 O13 O14 O15')
_LAST = (2, 4, 1, 7, 7, 'S14 V15 P12 S15 O9 X9 P13 O10 X10 P14 O11 X11 P15 O12 O13 O14 O15 X12 X13 X14 X15')
SCHED = (_EVEN, _ODD, _EVEN, _LAST)
FILLS = (('a0 a1', 'a2 a3'), ('', 'o0 o1'), ('o4', 'o2 o3'), ('', ''))
POS = ('QPKSVOX', 'QSKPVOX')

_NT = (((1,), (1,)), ((), ()))


def _dot(a, b):
    return jnp.dot(a, b, preferred_element_type=F32)


def _dot_nt(a, b):
    return lax.dot_general(a, b, _NT, preferred_element_type=F32)


def _iota(shape, dim):
    return lax.broadcasted_iota(jnp.int32, shape, dim)


def _rows(r0, n, align):
    if isinstance(r0, int):
        return slice(r0, r0 + n)
    return pl.ds(pl.multiple_of(r0, align), n)


def _ld(ref, t, r0, n):
    return pltpu.bitcast(ref.bitcast(U32)[t, _rows(r0 // 2, n // 2, 8), :], BF16)


def _st(ref, t, r0, val):
    ref[t, _rows(r0, val.shape[0], 16), :] = val


def _ktiles(ref, r0, n):
    parts = [_ld(ref, t, r0, n) for t in range(4)] + [_ld(ref, 4, r0, n)[:, 0:64]]
    return jnp.concatenate(parts, axis=1)


def _store_ktiles(ref, r0, val):
    for t in range(4):
        _st(ref, t, r0, val[:, 128 * t:128 * (t + 1)].astype(BF16))
    last = val[:, 512:576]
    _st(ref, 4, r0, jnp.concatenate([last, last], axis=1).astype(BF16))


def _store_transposed(ref, r0, blk):
    for t in range(4):
        _st(ref, t, r0, _xpose(blk[128 * t:128 * (t + 1), :]))
    _st(ref, 4, r0, _xpose(jnp.concatenate([blk[512:576, :], blk[512:576, :]], axis=0)))


def _xpose(x):
    return x.astype(F32).T.astype(BF16)


def _recip(x):
    r = pl.reciprocal(x, approx=True)
    return r * (2.0 - x * r)


def _hedgehog(p):
    sl = [p[8 * f:8 * f + 8, :] for f in range(DA)]
    mx = functools.reduce(jnp.maximum, sl)
    mn = functools.reduce(jnp.minimum, sl)
    cp = mx + jnp.log2(functools.reduce(jnp.add, [jnp.exp2(s - mx) for s in sl]))
    cn = mn - jnp.log2(functools.reduce(jnp.add, [jnp.exp2(mn - s) for s in sl]))
    return jnp.concatenate([jnp.exp2(s - cp) for s in sl] + [jnp.exp2(cn - s) for s in sl],
                           axis=0).astype(BF16)


def _kernel(axT_h, awqkv_h, wphi_h, awo_h, bxT_h, mem0_h, wq_h, wk_h, wv_h, woT_h,
            out_h,
            axT, awqkv, wphi, awo, bxT, mem0, wstage, woT_st,
            w2d, bdts, wT, kvacc, kvb, woTp, oTs, phiq, bx, wqkv_s, wo_s, fmask, outv,
            st_qkv, st_o, phi3, vt3, bhold, xhold, wh_s, ox_s,
            sem_in, sem_out):
    sem_s = sem_in.at[pl.ds(0, 6)]
    sem_ax = sem_in.at[pl.ds(6, N1)]
    sem_wo = sem_in.at[pl.ds(6 + N1, N1)]
    sem_w = sem_in.at[pl.ds(6 + 2 * N1, 2 * N1)]
    sem_bx = sem_in.at[pl.ds(6 + 4 * N1, N2 + 1)]

    def wdst(r0, n, t):
        return wstage.at[_rows(t * 3 * D + r0, n, 16)]

    def copy(src, dst, sem):
        pltpu.make_async_copy(src, dst, sem).start()

    def wait(dst, sem):
        pltpu.make_async_copy(dst, dst, sem).wait()

    def start_w(c):
        lo, hi = c * WCH, (c + 1) * WCH if c < N1 - 1 else 3 * D
        for t in range(2):
            for m, w_h in enumerate((wq_h, wk_h, wv_h)):
                a, b = max(lo, m * D), min(hi, (m + 1) * D)
                if a < b:
                    copy(w_h.bitcast(U32).at[pl.ds(a - m * D, b - a), pl.ds(8 * t, 8), :],
                         wdst(a, b - a, t), sem_w.at[2 * c + t])

    def wait_w(c, n):
        for t in range(2):
            wait(wdst(c * WCH, n, t), sem_w.at[2 * c + t])

    def start_ax(i):
        for b in range(2 * i, 2 * i + 2):
            copy(axT_h.at[:, pl.ds(128 * b, 128)], axT.at[b], sem_ax.at[i])

    def start_wo(i):
        copy(woT_h.at[pl.ds(4 * i, 4)], woT_st.at[pl.ds(4 * i, 4)], sem_wo.at[i])

    q_cols, k_cols, v_cols = pl.ds(0, 512), pl.ds(512, 640), pl.ds(2 * D, D)
    copy(wphi_h, wphi, sem_s.at[0])
    copy(awqkv_h.at[:, k_cols], awqkv.at[:, k_cols], sem_s.at[2])
    copy(awqkv_h.at[:, q_cols], awqkv.at[:, q_cols], sem_s.at[5])
    copy(awqkv_h.at[:, v_cols], awqkv.at[:, v_cols], sem_s.at[3])
    start_ax(0)
    for i in range(1, N1):
        start_ax(i)
        start_w(i - 1)
        start_wo(i - 1)
    start_w(N1 - 1)
    start_wo(N1 - 1)
    copy(awo_h, awo, sem_s.at[1])
    copy(mem0_h, mem0, sem_s.at[4])
    for b in range(N2 + 1):
        copy(bxT_h.at[:, pl.ds(min(b, N2 - 1) * T2, T2)], bxT.at[b], sem_bx.at[b])

    ri = _iota((80, 80), 0)
    ci = _iota((80, 80), 1)
    head_r = ((ri >= 32) & (ri < 64)) | (ri >= 72)
    head_c = ((ci >= 32) & (ci < 64)) | (ci >= 72)
    same = head_r == head_c
    vis = (ri >= 64) | (ci >= 64) | ((ci & 31) <= (ri & 31))
    scale = DB ** -0.5
    fmask[...] = jnp.where(same, jnp.where(vis, 0.0, -1e9 / scale), -jnp.inf).astype(F32)

    w2d[...] = jnp.zeros(w2d.shape, F32)
    kvacc[...] = jnp.zeros(kvacc.shape, F32)
    rj = _iota((GR, 256), 0) & 7
    cc = _iota((GR, 256), 1)
    wait(wphi, sem_s.at[0])
    eye32 = (_iota((H, H), 0) == _iota((H, H), 1)).astype(BF16)
    for d in range(DA):
        w2d[pl.ds(64 + d, H, stride=DA), 0:DA] = _dot_nt(eye32, wphi[d])
    w2b = w2d[...].astype(BF16)
    e2 = ((_iota((GR, 128), 0) >> 3) == _iota((GR, 128), 1)).astype(BF16)
    for g in range(NG):
        lo = (8 * g + rj) * DA
        for u, woff in enumerate((0, 64)):
            hd = cc + (128 * g + woff - 64)
            bdt = _dot_nt(e2, w2b[128 * g + woff:128 * g + woff + 256, :])
            bdt = jnp.where((hd >= lo) & (hd < lo + DA), bdt, 0.0).astype(BF16)
            for t in range(2):
                _st(bdts, 4 * g + 2 * u + t, 0, bdt[:, 128 * t:128 * (t + 1)])
    log2e = math.log2(math.e)
    for u, (base, coff) in enumerate(((2 * D, 512), (0, 0))):
        wait(awqkv.at[:, (k_cols, q_cols)[u]], sem_s.at[(2, 5)[u]])
        for g in range(NG):
            bdt = jnp.concatenate([_ld(bdts, 4 * g + 2 * u + t, 0, GR) for t in range(2)], axis=1)
            wfold = _dot_nt(bdt, awqkv[:, coff + 128 * g:coff + 128 * g + 256])
            _store_ktiles(wT, base + GR * g, wfold * log2e)

    s2 = wstage.reshape(2 * 3 * D * 8, DB)

    def relayout(c, n):
        for b in range(n // 16):
            r0 = c * WCH + b * 16
            for t in range(2):
                off = (t * 3 * D + r0) * 8
                if not isinstance(c, int):
                    off = pl.multiple_of(off, 128)
                sub = s2.at[pl.ds(off, 128)]
                for i in range(8):
                    u = sub[pl.ds(i, 16, stride=8), :]
                    lo = pltpu.bitcast(u << 16, F32).astype(BF16)
                    hi = pltpu.bitcast(u & jnp.uint32(0xFFFF0000), F32).astype(BF16)
                    _st(wqkv_s, 16 * t + 2 * i, r0, lo)
                    _st(wqkv_s, 16 * t + 2 * i + 1, r0, hi)

    def kv_update(g, vt, phi):
        r = _dot_nt(vt[0], phi[0]) + _dot_nt(vt[1], phi[1])
        for t, n in enumerate((128, 128, 32)):
            r0 = 160 * (3 * g + t)
            kvacc[r0:r0 + 160, 0:n] += r[:, 128 * t:128 * t + n]

    ones = jnp.ones((16, 128), F32)

    def hold(ref, val):
        for b in range(2):
            _st(ref, b, 0, val[b])

    def held(ref):
        return [_ld(ref, b, 0, ref.shape[1]) for b in range(2)]

    def xpose_bx(blk):
        _store_transposed(bx, blk * T2, _ld(bxT, blk, 0, D))

    def store_xposed(dst, r0, src, c0):
        for t in range(5):
            n = 128 if t < 4 else 64
            blk = src[:, c0 + 128 * t:c0 + 128 * t + n]
            if n == 64:
                blk = jnp.concatenate([blk, blk], axis=1)
            for kt in range(4):
                _st(dst, kt, r0 + 128 * t, _xpose(blk[128 * kt:128 * (kt + 1), :])[0:n])
            last = jnp.concatenate([blk[512:D, :], blk[512:D, :]], axis=0)
            _st(dst, 4, r0 + 128 * t, _xpose(last)[0:n])

    def b_weights(c, n):
        for hh in range(4):
            h = 4 * c + hh
            for t in range(4):
                _st(wo_s, t, h * DB, _xpose(_ld(woT_st, h, 128 * t, 128)))
        for pp_ in range(2):
            h = 4 * c + 2 * pp_
            last = jnp.concatenate([_ld(woT_st, h + j, 512, 64) for j in range(2)], axis=0)
            _st(wh_s, 2 * c + pp_, 0, _xpose(last))
        relayout(c, n)

    def wait_b(c, n):
        wait_w(c, n)
        wait(woT_st.at[pl.ds(4 * c, 4)], sem_wo.at[c])

    def proj(i, r0, f):
        w = _ktiles(wT, r0, GR)
        return [f(_dot(w, _ld(axT, 2 * i + b, 0, D))) for b in range(T1 // 128)]

    def pq(i, g):
        for b, phi in enumerate(proj(i, GR * g, _hedgehog)):
            _st(phiq, 2 * i + b, 288 * g, phi)

    def phase1(i, carry):
        first = isinstance(i, int)
        wait(axT.at[pl.ds(2 * i, 2)], sem_ax.at[i])

        def pk(g):
            return proj(i, 2 * D + GR * g, _hedgehog)

        def vt(g):
            return proj(i, D + GR * g,
                        lambda v: jnp.concatenate([v, ones], axis=0).astype(BF16))

        if first:
            wait(awqkv.at[:, v_cols], sem_s.at[3])
            store_xposed(wT, D, awqkv, 2 * D)
            ks = [pk(g) for g in range(NG)]
            for g in range(PQA):
                pq(0, g)
            for g in range(3):
                kv_update(g, vt(g), ks[g])
            k = ks[3]
        else:
            wait_b(i - 1, WCH)
            kv_update(3, held(vt3), held(phi3))
            qs = [(i - 1, g) for g in range(PQA, NG)] + [(i, g) for g in range(PQA)]
            k = pk(0)
            for g in range(3):
                v = vt(g)
                pq(*qs[g])
                kn = pk(g + 1)
                if g == 2:
                    pq(*qs[3])
                kv_update(g, v, k)
                k = kn
            b_weights(i - 1, WCH)
        hold(phi3, k)
        hold(vt3, vt(3))
        return carry

    phase1(0, 0)
    lax.fori_loop(1, N1, phase1, 0)
    w_last = 3 * D - (N1 - 1) * WCH
    wait_b(N1 - 1, w_last)
    wait(awo, sem_s.at[1])
    wait(mem0, sem_s.at[4])
    wait(bxT.at[0], sem_bx.at[0])
    xpose_bx(0)
    store_xposed(woTp, 0, awo, 0)
    own = (_iota((160, 128), 0) & 7) == (_iota((160, 128), 1) & 7)

    def kv_finish(g):
        for t in range(3 * g, 3 * g + 3):
            kv = jnp.concatenate(
                [kvacc[pl.ds(160 * t + d, 8, stride=DA), :] for d in range(DA)]
                + [kvacc[160 * t + GR:160 * (t + 1), :]], axis=0)
            _st(kvb, t, 0, jnp.where(own, kv, 0.0).astype(BF16))

    for g in range(3):
        kv_finish(g)
    for g in range(PQA, NG):
        pq(N1 - 1, g)
    kv_update(3, held(vt3), held(phi3))
    kv_finish(3)
    b_weights(N1 - 1, w_last)

    cexp = scale * math.log2(math.e)

    def stack(a, b):
        return jnp.concatenate([a[0], b[0], a[1], b[1]], axis=0).astype(BF16)

    def scores(q2, k2):
        s = _dot_nt(q2, k2)
        fm = fmask[...]
        s = jnp.where(fm == 0.0, s, fm)
        m = jnp.max(s, axis=1, keepdims=True)
        p = jnp.exp2((s - m) * cexp)
        l = jnp.sum(p, axis=1, keepdims=True)
        return p.astype(BF16), _recip(l)

    def out_proj(lhs, hp):
        return jnp.concatenate(
            [_dot(lhs, _ld(wo_s, t, 256 * hp, 256)) for t in range(4)], axis=1)

    def b_step(lhs, seg, fill_mid, fill_end):
        first = seg % 2 == 0
        qk, vv, pp, oo = {}, {}, {}, {}
        acc, accm, accx = [None], [None], [None]

        def add(a, c):
            a[0] = c if a[0] is None else a[0] + c

        def proj(hp, t):
            idx = 6 * hp + t
            a = _dot(lhs, _ld(wqkv_s, 2 * hp + t % 2, D * (t // 2), D))
            if first:
                st_qkv[idx] = a[32:40]
                return a[0:32], a[40:48]
            return jnp.concatenate([st_qkv[idx], a[8:32]], axis=0), a[0:8]

        def st_s(hp):
            if 0 <= hp < 16:
                pp[hp] = scores(*qk.pop(hp))

        def st_pv(hp):
            if 0 <= hp < 16:
                p, rl = pp.pop(hp)
                o = _dot(p, vv.pop(hp)) * rl
                halves = []
                for j, (ox, om) in enumerate(((o[0:32], o[64:72]), (o[32:64], o[72:80]))):
                    if first:
                        st_o[2 * hp + j] = ox[24:32]
                        halves.append(jnp.concatenate([ox[0:24], om], axis=0))
                    else:
                        halves.append(jnp.concatenate([st_o[2 * hp + j], ox, om], axis=0))
                for j in range(2):
                    _st(ox_s, 2 * hp + j, SEG * seg, o[32 * j:32 * (j + 1)].astype(BF16))
                oo[hp] = (jnp.concatenate(halves, axis=1).astype(BF16), o[64:80].astype(BF16))

        def st_x(hp):
            if seg == 3 and 0 <= hp < 16:
                for h in (2 * hp, 2 * hp + 1):
                    add(accx, _dot_nt(_ld(woT_st, h, 512, 64), _ld(ox_s, h, 0, T2)))
                xdone.add(hp)

        def st_out(hp):
            if 0 <= hp < 16:
                lo_, om = oo.pop(hp)
                add(acc, out_proj(lo_, hp))
                add(accm, _dot(om, _ld(wh_s, hp, 0, DB)))

        ls, lp, lv, lo, lx, tail = SCHED[seg]
        xdone = set()
        qs = {}

        def st_v(hp):
            if 0 <= hp < 16:
                vv[hp] = stack(proj(hp, 4), proj(hp, 5))

        def st_q(t):
            qs[t] = stack(proj(t, 0), proj(t, 1))

        def st_k(t):
            qk[t] = (qs.pop(t), stack(proj(t, 2), proj(t, 3)))

        for t in range(16):
            for c in POS[seg % 2]:
                dict(Q=lambda: st_q(t), K=lambda: st_k(t), S=lambda: st_s(t - ls),
                     P=lambda: st_pv(t - lp), V=lambda: st_v(t - lv),
                     O=lambda: st_out(t - lo), X=lambda: st_x(t - lx))[c]()
        for tok in tail.split():
            if tok == "M":
                for f in fill_mid:
                    f()
            else:
                dict(S=st_s, P=st_pv, V=st_v, O=st_out, X=st_x)[tok[0]](int(tok[1:]))
        assert not (qk or vv or pp or oo)
        if seg == 3:
            assert len(xdone) == 16
            xhold[...] = accx[0]
        for f in fill_end:
            f()
        a, am = acc[0], accm[0]
        n = a.shape[0] - MEM
        mlast = am[0:8] + pltpu.roll(am[8:16], 64, 1)
        mem = jnp.concatenate([a[n:], mlast[:, 0:64]], axis=1)
        return a[0:n], mem.astype(BF16).astype(F32)

    def b_pair(r0, seg, mem, fills):
        x48 = _ktiles(bx, r0, 48).astype(F32)
        x16 = _ktiles(bx, r0 + 48, 16).astype(F32)
        lhs = jnp.concatenate([x48[0:40], mem], axis=0).astype(BF16)
        b1, mem = b_step(lhs, seg, *fills[0])
        lhs = jnp.concatenate([mem, x48[40:48], x16], axis=0).astype(BF16)
        b2, mem = b_step(lhs, seg + 1, *fills[1])
        return jnp.concatenate([b1, b2], axis=0), mem

    def a_attn(i, g):
        kv = jnp.concatenate([_ld(kvb, 3 * g + t, 0, 160) for t in range(3)], axis=1)
        r = _dot(kv[:, 0:288], _ld(phiq, i, 288 * g, 288))
        rden = 1.0 / (r[GR:GR + 8] + 1e-06)
        for d in range(DA):
            oTs[pl.ds(GR * g + d, 8, stride=DA), :] = r[8 * d:8 * d + 8] * rden

    def a_out(r0, c):
        n = 128 if c < 4 else 64
        oT = _dot(_ktiles(woTp, 128 * c, n), oTs[...].astype(BF16))
        if n == 64:
            oT = jnp.concatenate([oT, oT], axis=0)
        outv[pl.ds(r0, T2), 128 * c:128 * c + n] = oT.T[:, 0:n].astype(BF16)

    def out_copy(i):
        rows = pl.ds(i * T2 if isinstance(i, int) else pl.multiple_of(i * T2, T2), T2)
        return pltpu.make_async_copy(outv.at[rows], out_h.at[rows], sem_out.at[i])

    def flush_b(i):
        outv[_rows(i * T2 + 64, 64, 64), D:D + 512] = bhold[...].astype(BF16)
        xt = xhold[...]
        xt = jnp.concatenate([xt, xt], axis=0).T
        outv[_rows(i * T2, T2, T2), D + 512:2 * D] = xt[:, 64:128].astype(BF16)

    def main(i, mem):
        wait(bxT.at[i + 1], sem_bx.at[i + 1])
        r0 = pl.multiple_of(i * T2, T2)
        flush_b(jnp.maximum(i - 1, 0))
        aa = [functools.partial(a_attn, i, g) for g in range(NG)]
        ao = [functools.partial(a_out, r0, c) for c in range(5)]
        fl = [[[dict(a=aa, o=ao)[t[0]][int(t[1])] for t in part.split()] for part in st]
              for st in FILLS]
        b1, mem = b_pair(r0, 0, mem, fl[0:2])
        outv[pl.ds(r0, 64), D:D + 512] = b1.astype(BF16)
        xpose_bx(i + 1)
        b2, mem = b_pair(r0 + 64, 2, mem, fl[2:4])
        bhold[...] = b2

        @pl.when(i > 0)
        def _():
            out_copy(i - 1).start()

        return mem

    bhold[...] = jnp.zeros(bhold.shape, F32)
    xhold[...] = jnp.zeros(xhold.shape, F32)
    lax.fori_loop(0, N2, main, mem0[...].astype(F32))
    flush_b(N2 - 1)
    out_copy(N2 - 1).start()
    for i in range(N2):
        out_copy(i).wait()


@functools.partial(jax.jit, static_argnames=("B_seg_len",))
def pallas_concat_heads__linear_kernel_hedgehog__memory_aug_recurrent_mem_tr__prompt_kernel(
    A_x: jax.Array,
    A_wqkv: jax.Array,
    A_w_phi: jax.Array,
    A_wo: jax.Array,
    B_x: jax.Array,
    B_mem0: jax.Array,
    B_Wq: jax.Array,
    B_Wk: jax.Array,
    B_Wv: jax.Array,
    B_Wo: jax.Array,
    B_seg_len: int,
):
    assert int(B_seg_len) == SEG
    assert A_x.shape == (1, S, D) and B_x.shape == (1, S, D)
    args = (
        A_x.reshape(S, D).T,
        A_wqkv,
        jnp.transpose(A_w_phi, (1, 2, 0)),
        A_wo,
        B_x.reshape(S, D).T,
        B_mem0.reshape(MEM, D),
        B_Wq,
        B_Wk,
        B_Wv,
        jnp.transpose(B_Wo, (0, 2, 1)),
    )
    hbm = pl.BlockSpec(memory_space=pltpu.HBM)
    out = pl.pallas_call(
        _kernel,
        out_shape=jax.ShapeDtypeStruct((S, 2 * D), BF16),
        in_specs=[hbm] * len(args),
        out_specs=hbm,
        scratch_shapes=[
            pltpu.VMEM((S // 128, D, 128), BF16),
            pltpu.VMEM((D, 3 * D), BF16),
            pltpu.VMEM((DA, DA, H), BF16),
            pltpu.VMEM((D, D), BF16),
            pltpu.VMEM((N2 + 1, D, T2), BF16),
            pltpu.VMEM((MEM, D), BF16),
            pltpu.VMEM((2 * 3 * D, 8, DB), U32),
            pltpu.VMEM((H, D, DB), BF16),
            pltpu.VMEM((704, 128), F32),
            pltpu.VMEM((4 * NG, GR, 128), BF16),
            pltpu.VMEM((5, 3 * D, 128), BF16),
            pltpu.VMEM((NG * 3 * 160, 128), F32),
            pltpu.VMEM((NG * 3, 160, 128), BF16),
            pltpu.VMEM((5, D, 128), BF16),
            pltpu.VMEM((D, T2), F32),
            pltpu.VMEM((N2, 2 * D, T2), BF16),
            pltpu.VMEM((5, S + T2, 128), BF16),
            pltpu.VMEM((H, 3 * D, DB), BF16),
            pltpu.VMEM((4, H * DB, 128), BF16),
            pltpu.VMEM((80, 80), F32),
            pltpu.VMEM((S, 2 * D), BF16),
            pltpu.VMEM((96, 8, 128), F32),
            pltpu.VMEM((32, 8, 128), F32),
            pltpu.VMEM((2, 288, 128), BF16),
            pltpu.VMEM((2, 160, 128), BF16),
            pltpu.VMEM((64, 512), F32),
            pltpu.VMEM((64, T2), F32),
            pltpu.VMEM((H // 2, DB, 128), BF16),
            pltpu.VMEM((H, T2, DB), BF16),
            pltpu.SemaphoreType.DMA((6 + 4 * N1 + N2 + 1,)),
            pltpu.SemaphoreType.DMA((N2,)),
        ],
        compiler_params=pltpu.CompilerParams(
            vmem_limit_bytes=100 * 1024 * 1024,
            disable_bounds_checks=True,
            disable_semaphore_checks=True,
        ),
    )(*args)
    return out.reshape(1, S, 2 * D)
```
